```python
import jax
import jax.numpy as jnp

def _softmax(x, axis=-1):
    return jax.nn.softmax(x, axis=axis)
def _gelu(x):
    return jax.nn.gelu(x, approximate=True)
def _silu(x):
    return jax.nn.silu(x)
def _sigmoid(x):
    return jax.nn.sigmoid(x)
def _layernorm(x, axis=-1, eps=1e-5):
    m = jnp.mean(x, axis=axis, keepdims=True)
    v = jnp.var(x, axis=axis, keepdims=True)
    return (x - m) / jnp.sqrt(v + eps)
def _scatter_add(tgt, idx, src, axis=0):
    return tgt.at[idx].add(src)
def _segment_sum(src, seg, n):
    return jax.ops.segment_sum(src, seg, n)
class _Rng:
    def __init__(self, key):
        self._k = key
    def _next(self):
        self._k, sub = jax.random.split(self._k)
        return sub
    def normal(self, shape):
        return jax.random.normal(self._next(), shape, dtype=jnp.bfloat16)
    def randint(self, lo, hi, shape):
        return jax.random.randint(self._next(), shape, lo, hi, dtype=jnp.int32)
    def uniform(self, shape, lo=0.0, hi=1.0):
        return jax.random.uniform(self._next(), shape, jnp.bfloat16, lo, hi)
    def permutation(self, n):
        return jax.random.permutation(self._next(), n)


kernel_name = 'standalone__gqa_softmax__near_ridge'

def setup_inputs():
    _rng = _Rng(jax.random.key(int.from_bytes(__import__("os").urandom(4), "little")))
    _w = (lambda a: (lambda t: t.astype(jnp.bfloat16) if jnp.issubdtype(t.dtype, jnp.floating) else t)(jnp.asarray(a)))
    B, Hq, Hkv, Sq, Sk, D = 16, 32, 32, 848, 512, 192
    return {
        "q": _w((lambda *s: _rng.normal(s) * 0.05)(B, Hq, Sq, D)),
        "k": _w((lambda *s: _rng.normal(s) * 0.05)(B, Hkv, Sk, D)),
        "v": _w((lambda *s: _rng.normal(s) * 0.05)(B, Hkv, Sk, D)),
    }

def reference(q, k, v):
    B, Hq, Sq, D = q.shape
    Hkv = k.shape[1]
    rep = Hq // Hkv
    k = jnp.repeat(k, rep, axis=1)
    v = jnp.repeat(v, rep, axis=1)
    scale = D ** -0.5
    scores = jnp.einsum("bhqd,bhkd->bhqk", q, k) * scale
    p = _softmax(scores, axis=-1)
    return jnp.einsum("bhqk,bhkd->bhqd", p, v)
```

```python
import math

import jax
import jax.numpy as jnp
import jax.experimental.pallas as pl
import jax.experimental.pallas.tpu as pltpu

_HEADS_PER_STEP = 4


def _attention_kernel(q_ref, k_ref, v_ref, o_ref, *, rep):
    d = q_ref.shape[1]
    c = d ** -0.5 * math.log2(math.e)
    for h in range(q_ref.shape[0]):
        kk = k_ref[h // rep].T
        s = jnp.dot(kk, q_ref[h], preferred_element_type=jnp.float32)
        m = jnp.max(s, axis=0, keepdims=True)
        p = jnp.exp2((s - m) * c)
        l = jnp.sum(p, axis=0, keepdims=True)
        o = jnp.dot(v_ref[h // rep], p.astype(v_ref.dtype),
                    preferred_element_type=jnp.float32)
        o_ref[h] = (o * (1.0 / l)).astype(o_ref.dtype)


@jax.jit
def pallas_standalone__gqa_softmax__near_ridge_kernel(
    q: jax.Array,
    k: jax.Array,
    v: jax.Array,
):
    B, Hq, Sq, D = q.shape
    Hkv, Sk = k.shape[1], k.shape[2]
    rep = Hq // Hkv
    hb = _HEADS_PER_STEP * rep
    qt = jnp.swapaxes(q, 2, 3).reshape(B * Hq, D, Sq)
    kt = jnp.swapaxes(k, 2, 3).reshape(B * Hkv, D, Sk)
    vt = jnp.swapaxes(v, 2, 3).reshape(B * Hkv, D, Sk)

    def kernel_function(*refs):
        _attention_kernel(*refs, rep=rep)

    ot = pl.pallas_call(
        kernel_function,
        grid=(B * Hq // hb,),
        in_specs=[
            pl.BlockSpec((hb, D, Sq), lambda i: (i, 0, 0)),
            pl.BlockSpec((hb // rep, D, Sk), lambda i: (i, 0, 0)),
            pl.BlockSpec((hb // rep, D, Sk), lambda i: (i, 0, 0)),
        ],
        out_specs=pl.BlockSpec((hb, D, Sq), lambda i: (i, 0, 0)),
        out_shape=jax.ShapeDtypeStruct((B * Hq, D, Sq), q.dtype),
        compiler_params=pltpu.CompilerParams(
            dimension_semantics=("parallel",),
            vmem_limit_bytes=100 * 1024 * 1024,
        ),
    )(qt, kt, vt)
    return jnp.swapaxes(ot.reshape(B, Hq, D, Sq), 2, 3)
```

```python
import functools
import jax, jax.numpy as jnp, numpy as np
from jax import lax
from jax.experimental import pallas as pl
from jax.experimental.pallas import tpu as pltpu
import math

def make(G=4, vmem=100, flags=None, nb=2, ch=32, la=3, kpos=(0,1,2,3), vpos=(2,3,4,5), nobc=True, tq=3, tp=5, tmode=2, opin=1, dpin=3, norm_p=False):
    qc=128
    nk=G
    def kern(z_ref,q_hbm,k_hbm,v_hbm,o_hbm,*sp):
        sp=list(sp); take=lambda n:[sp.pop(0) for _ in range(n)]
        q_in,k_in,v_in=take(3); o_out=take(G)
        k_s=take(nk); kt_s=take(nk); v_s=take(nk); s_s=take(nb); pt_s=take(2); rt_s=take(2); sem=take(1)[0]
        NH,D,Sq=q_hbm.shape; Sk=k_hbm.shape[2]
        c=D**-0.5*math.log2(math.e)
        nt=Sq//qc; nkb=Sk//128; s_t=nt*qc; n_t=Sq-s_t
        NG=NH//G
        cnt=[0]
        f32=lambda x: pltpu.bitcast(x,jnp.float32)
        u32=lambda x: pltpu.bitcast(x,jnp.uint32)
        bf=lambda x: pltpu.bitcast(x,jnp.bfloat16)
        def Z():
            cnt[0]+=1
            return z_ref[cnt[0]%z_ref.shape[0]]
        def in_copies(g,half):
            b=g*G; o=half*G
            return [pltpu.make_async_copy(k_hbm.at[pl.ds(b+1,G-1)],k_in.at[pl.ds(o,G-1)],sem.at[half]),
                    pltpu.make_async_copy(k_hbm.at[jnp.minimum(b+G,NH-1)],k_in.at[o+G-1],sem.at[half]),
                    pltpu.make_async_copy(q_hbm.at[pl.ds(b,G)],q_in.at[pl.ds(o,G)],sem.at[half]),
                    pltpu.make_async_copy(v_hbm.at[pl.ds(b,G)],v_in.at[pl.ds(o,G)],sem.at[half])]
        def out_all(half):
            return pltpu.make_async_copy(q_in.at[pl.ds(0,G)],o_hbm.at[pl.ds(0,G)],sem.at[2+half])
        def kprep(dst,src,j):
            x=k_in[src,:,j*128:(j+1)*128]
            k_s[dst][0,j*64:(j+1)*64,:]=u32(x.T)
            kt_s[dst][0,:,j*128:(j+1)*128]=u32(x)
        def vprep(dst,src,j):
            v_s[dst][0,:,j*128:(j+1)*128]=u32(v_in[src,:,j*128:(j+1)*128])
        c0=pltpu.make_async_copy(k_hbm.at[0],k_in.at[G],sem.at[1]); c0.start()
        for d in in_copies(0,0): d.start()
        c0.wait()
        for j in range(nkb): kprep(0,G,j)

        def body(it,_):
            base=it*G; half=it%2; off=half*G
            cnt[0]=0
            for d in in_copies(jnp.minimum(it+1,NG-1),1-half): d.start()
            for d in in_copies(it,half): d.wait()
            @pl.when(it>=2)
            def _w(): out_all(half).wait()
            for j in range(nkb): vprep(0,off,j)
            units=[(h,s) for h in range(G) for s in range(0,s_t,qc)]
            pins={}
            def pin(i,fn): pins.setdefault(i,[]).append(fn)
            def qk(i):
                h,s0=units[i]
                sb=s_s[i%nb]
                z=Z()
                qt=q_in[off+h,:,s0:s0+qc]
                r=Sk//2
                m=None
                for j in range(2):
                    s=jnp.dot(bf(k_s[h][z,j*r//2:(j+1)*r//2,:]),qt,preferred_element_type=jnp.float32)
                    mm=jnp.max(s.reshape(r//8,8,qc),axis=0)
                    m=mm if m is None else jnp.maximum(m,mm)
                    sb[0,j*r:(j+1)*r,:]=s
                return jnp.broadcast_to(jnp.max(m,axis=0,keepdims=True),(8,qc))
            def softmax(i,m):
                h,s0=units[i]
                t=i%nt
                sb=s_s[i%nb]
                z=Z()
                for j in range(nkb):
                    if t==kpos[j]:
                        kprep((h+1)%G,off+h,j)
                        pin(i,lambda z,j=j: f32(k_s[(h+1)%G][z,j*64:j*64+8,0:128]))
                        pin(i,lambda z,j=j: f32(kt_s[(h+1)%G][z,0:8,j*128:(j+1)*128]))
                    if t==vpos[j] and h+1<G:
                        vprep(h+1,off+h+1,j)
                        pin(i,lambda z,j=j: f32(v_s[h+1][z,0:8,j*128:(j+1)*128]))
                for n_,fn in enumerate(pins.pop(i,[])):
                    sb[0,Sk+8*n_:Sk+8*n_+8,:]=fn(z)
                l=None
                nch=Sk//ch
                ld=lambda t: sb[z,t*ch:(t+1)*ch,:].reshape(ch//8,8,qc)
                order=list(range(nch))[::-1]
                pend=[ld(order[t]) for t in range(la)]
                ps={}
                for tt in range(nch):
                    t=order[tt]
                    s=pend.pop(0)
                    p=jnp.exp2((s-m)*c)
                    ll=jnp.sum(p,axis=0)
                    l=ll if l is None else l+ll
                    ps[t]=p.reshape(ch,qc)
                    if tt+la<nch:
                        sb[0,t*ch:t*ch+8,:]=l
                        pend.append(ld(order[tt+la]))
                l=jnp.sum(l,axis=0,keepdims=True)
                return 1.0/l,jnp.concatenate([ps[t] for t in range(nch)],axis=0).astype(jnp.bfloat16)
            def pv(i,r,p):
                h,s0=units[i]
                z=Z()
                o=jnp.dot(bf(v_s[h][z]),p,preferred_element_type=jnp.float32)
                o_out[h][half,:,s0:s0+qc]=(o*r).astype(jnp.bfloat16)
                if i%nt==nt-1:
                    pin(i+1+opin,lambda z: f32(o_out[h][half,0:16,0:128]))
                    pltpu.make_async_copy(o_out[h].at[half],o_hbm.at[base+h],sem.at[2+half]).start()
                    if dpin is not None:
                        def fn(z):
                            o_out[h][2+z,0:16,0:128]=jnp.zeros((16,128),jnp.bfloat16)
                            return f32(o_out[h][2,0:16,0:128])
                        pin(i+1+dpin,fn)
            def qk_tail(h,i):
                z=Z()
                qq=q_in[off+h,:,s_t:Sq].T
                s=jnp.dot(qq,bf(kt_s[h][z]),preferred_element_type=jnp.float32)
                m=jnp.max(s,axis=1,keepdims=True)
                p=jnp.exp2((s-m)*c)
                l=jnp.sum(p,axis=1,keepdims=True)
                if tmode==2 and not norm_p:
                    rt_s[h%2][0]=jnp.broadcast_to(1.0/l,(n_t,128))
                    pin(i,lambda z: rt_s[h%2][z,0:8,:])
                else:
                    p=p*(1.0/l)
                pt_s[h%2][0]=u32(p.astype(jnp.bfloat16))
                pin(i,lambda z: f32(pt_s[h%2][z,0:8,0:128]))
            def pv_tail(h):
                z=Z()
                p=bf(pt_s[h%2][z])
                vt=bf(v_s[h][z])
                nt_=(((1,),(1,)),((),()))
                if tmode==2:
                    o=lax.dot_general(p,vt,nt_,preferred_element_type=jnp.float32)
                    if not norm_p:
                        r=rt_s[h%2][z]
                        o=o*jnp.concatenate([r,r[:,:D-128]],axis=1)
                    o_out[h][half,:,s_t:Sq]=o.astype(jnp.bfloat16).T
                else:
                    o=lax.dot_general(vt,p,nt_,preferred_element_type=jnp.float32)
                    o_out[h][half,:,s_t:Sq]=o.astype(jnp.bfloat16)
            N=len(units)
            prev=None
            for i in range(N+1):
                h,t=i//nt,i%nt
                if i<N: m=qk(i)
                if i==0: qk_tail(0,1)
                if i>=1: pv(i-1,*prev)
                if i<N: prev=softmax(i,m)
                if i<N and h>0 and t==tq: qk_tail(h,i+1)
                if i<N and t==tp: pv_tail(h)
            return _
        lax.fori_loop(0,NG,body,0)
        for d in in_copies(0,NG%2): d.wait()
        out_all(0).wait(); out_all(1).wait()
    @jax.jit
    def f(q,k,v):
        B,H,Sq,D=q.shape; Sk=k.shape[2]
        qt=jnp.swapaxes(q,2,3).reshape(B*H,D,Sq)
        kt=jnp.swapaxes(k,2,3).reshape(B*H,D,Sk)
        vt=jnp.swapaxes(v,2,3).reshape(B*H,D,Sk)
        V=pltpu.VMEM; bf=jnp.bfloat16
        o=pl.pallas_call(kern,
            in_specs=[pl.BlockSpec(memory_space=pltpu.SMEM)]+[pl.BlockSpec(memory_space=pl.ANY)]*3,
            out_specs=pl.BlockSpec(memory_space=pl.ANY),
            out_shape=jax.ShapeDtypeStruct((B*H,D,Sq),q.dtype),
            scratch_shapes=[V((2*G,D,Sq),bf),V((2*G,D,Sk),bf),V((2*G,D,Sk),bf)]+[V((3,D,Sq),bf)]*G+[V((1,Sk//2,D),jnp.uint32)]*nk+[V((1,D//2,Sk),jnp.uint32)]*(2*nk)+[V((1,Sk+64,qc),jnp.float32)]*nb+[V((1,(Sq%qc)//2,Sk),jnp.uint32)]*2+[V((1,Sq%qc,128),jnp.float32)]*2+[pltpu.SemaphoreType.DMA((4,))],
            compiler_params=pltpu.CompilerParams(vmem_limit_bytes=vmem*1024*1024,flags=flags,disable_bounds_checks=nobc),
            )(np.zeros((512,),np.int32),qt,kt,vt)
        return jnp.swapaxes(o.reshape(B,H,D,Sq),2,3)
    return f


_impl = make(G=8)


@jax.jit
def pallas_standalone__gqa_softmax__near_ridge_kernel(q: jax.Array, k: jax.Array, v: jax.Array):
    return _impl(q, k, v)
```

```python
import math

import jax
import jax.numpy as jnp
from jax import lax
import jax.experimental.pallas as pl
import jax.experimental.pallas.tpu as pltpu

LANES = 128
NT_DIMS = (((1,), (1,)), ((), ()))

DEFAULTS = dict(
    group=16,
    ramp=2,
    chunk=32,
    ahead=4,
    tail_ahead=3,
    k_at=(0, 1, 3, 4),
    v_at=(0, 2, 3, 4),
    q_at=5,
    dma_lag=1,
)
TAIL_QK_AT = (0, 1)
TAIL_PV_AT = (4, 5)


def _as_u32(x):
    return pltpu.bitcast(x, jnp.uint32)


def _as_f32(x):
    return pltpu.bitcast(x, jnp.float32)


def _as_bf16(x):
    return pltpu.bitcast(x, jnp.bfloat16)


def _attention_kernel(q_hbm, k_hbm, v_hbm, o_hbm,
                      q_in, k_in, v_in, o_out, k_s, kt_s, v_s, s_s,
                      qt_s, st_s, mt_s, pt_s, in_sem, out_sem,
                      *, group, ramp, chunk, ahead, tail_ahead,
                      k_at, v_at, q_at, dma_lag):
    n_heads, d, sq = q_hbm.shape
    sk = k_hbm.shape[2]
    c = d ** -0.5 * math.log2(math.e)
    n_units = sq // LANES
    tail0 = n_units * LANES
    n_tail = sq - tail0
    key_blocks = sk // LANES
    ramp_heads = group * ramp
    n_groups = (n_heads - ramp_heads) // group

    def start_inputs(head, n, slot, sem):
        last = jnp.minimum(head + n, n_heads - 1)
        pltpu.make_async_copy(k_hbm.at[last], k_in.at[slot + n - 1], sem).start()
        if n > 1:
            pltpu.make_async_copy(k_hbm.at[pl.ds(head + 1, n - 1)],
                                  k_in.at[pl.ds(slot, n - 1)], sem).start()
        for src, dst in ((q_hbm, q_in), (v_hbm, v_in)):
            pltpu.make_async_copy(src.at[pl.ds(head, n)],
                                  dst.at[pl.ds(slot, n)], sem).start()

    def wait_inputs(n, slot, sem):
        for buf in (k_in, q_in, v_in):
            filled = buf.at[pl.ds(slot, n)]
            pltpu.make_async_copy(filled, filled, sem).wait()

    def output_copy(h, slot, head):
        return pltpu.make_async_copy(o_out[h].at[slot], o_hbm.at[head],
                                     out_sem.at[slot])

    def wait_outputs(n, slot, head):
        for h in range(n):
            output_copy(h, slot, head + h).wait()

    def prepare_k(h, slot, j):
        kt = k_in[slot, :, j * LANES:(j + 1) * LANES]
        k_s[h][0, j * LANES // 2:(j + 1) * LANES // 2, :] = _as_u32(kt.T)
        if h == 0:
            kt_s[0, :, j * LANES:(j + 1) * LANES] = _as_u32(kt)

    def prepare_v(h, slot, j):
        v_s[h][0, :, j * LANES:(j + 1) * LANES] = _as_u32(
            v_in[slot, :, j * LANES:(j + 1) * LANES])

    def run_group(it, n, head0, slot0, out_slot):
        n_zeros = 0

        def zero():
            nonlocal n_zeros
            n_zeros += 1
            return lax.shift_right_logical(it + n_zeros, 24)

        before_softmax, before_qk_end = {}, {}

        def pin(where, unit, load):
            where.setdefault(unit, []).append(load)

        def qk(u):
            h, t = divmod(u, n_units)
            buf, z = s_s[u % 2], zero()
            qt = q_in[slot0 + h, :, t * LANES:(t + 1) * LANES]
            half, early = sk // 2, 160
            parts, m = [], None
            for j in range(2):
                k = _as_bf16(k_s[h][z, j * half // 2:(j + 1) * half // 2, :])
                s = jnp.dot(k, qt, preferred_element_type=jnp.float32)
                mj = jnp.max(s.reshape(half // 8, 8, LANES), axis=0)
                m = mj if m is None else jnp.maximum(m, mj)
                buf[0, j * half:j * half + early, :] = s[:early]
                parts.append(s[early:])
            for i, load in enumerate(before_qk_end.pop(u, [])):
                buf[z, sk + 32 + 8 * i:sk + 40 + 8 * i, :] = load(z)
            for j in range(2):
                buf[0, j * half + early:(j + 1) * half, :] = parts[j]
            return jnp.broadcast_to(jnp.max(m, axis=0, keepdims=True), (8, LANES))

        def prepare_next_head(u):
            h, t = divmod(u, n_units)
            nxt = (h + 1) % n
            for j in range(key_blocks):
                if t == k_at[j]:
                    prepare_k(nxt, slot0 + h, j)
                    pin(before_softmax, u, lambda z, j=j: _as_f32(
                        k_s[nxt][z, j * LANES // 2:j * LANES // 2 + 8, 0:LANES]))
                    if nxt == 0:
                        pin(before_softmax, u, lambda z, j=j: _as_f32(
                            kt_s[z, 0:8, j * LANES:(j + 1) * LANES]))
                if t == v_at[j] and nxt:
                    prepare_v(nxt, slot0 + nxt, j)
                    pin(before_qk_end, u + 1, lambda z, j=j: _as_f32(
                        v_s[nxt][z, 0:8, j * LANES:(j + 1) * LANES]))
            if t == q_at and nxt:
                prepare_tail_q(nxt)
                pin(before_softmax, u,
                    lambda z: _as_f32(qt_s[nxt % 2][z, 0:8, 0:LANES]))

        def softmax(u, m):
            buf, z = s_s[u % 2], zero()
            for i, load in enumerate(before_softmax.pop(u, [])):
                buf[0, sk + 8 * i:sk + 8 * i + 8, :] = load(z)
            starts = list(range(0, sk, chunk))[::-1]

            def scores(i):
                return buf[z, starts[i]:starts[i] + chunk, :]

            loaded = [scores(i) for i in range(ahead)]
            p, l = [], None
            for i in range(len(starts)):
                s = loaded.pop(0).reshape(chunk // 8, 8, LANES)
                e = jnp.exp2((s - m) * c)
                li = jnp.sum(e, axis=0)
                l = li if l is None else l + li
                p.insert(0, e.reshape(chunk, LANES))
                if i + ahead < len(starts):
                    buf[0, starts[i]:starts[i] + 8, :] = l
                    loaded.append(scores(i + ahead))
            l = jnp.sum(l, axis=0, keepdims=True)
            return jnp.concatenate(p, axis=0).astype(jnp.bfloat16), 1.0 / l

        def pv(u, p, inv_l):
            h, t = divmod(u, n_units)
            o = jnp.dot(_as_bf16(v_s[h][zero()]), p,
                        preferred_element_type=jnp.float32)
            o_out[h][out_slot, :, t * LANES:(t + 1) * LANES] = (
                o * inv_l).astype(o_hbm.dtype)
            if t == n_units - 1:
                output_copy(h, out_slot, head0 + h).start()

                def after_dma_start(z):
                    o_out[h][z, 0:16, 0:LANES] = jnp.zeros((16, LANES), o_hbm.dtype)
                    return _as_f32(o_out[h][0, 0:16, 0:LANES])

                pin(before_softmax, u + 1 + dma_lag, after_dma_start)

        def prepare_tail_q(h):
            qt_s[h % 2][0] = _as_u32(q_in[slot0 + h, :, tail0:sq].T)

        def tail_qk(h, part, u):
            z, w = zero(), sk // 2
            if h == 0:
                kt = _as_bf16(kt_s[z, :, part * w:(part + 1) * w])
            else:
                kt = k_in[slot0 + h - 1, :, part * w:(part + 1) * w]
            s = jnp.dot(_as_bf16(qt_s[h % 2][z]), kt,
                        preferred_element_type=jnp.float32)
            st_s[0, 0:n_tail, part * w:(part + 1) * w] = s
            m = s[:, 0:LANES]
            for j in range(LANES, w, LANES):
                m = jnp.maximum(m, s[:, j:j + LANES])
            if part == 0:
                mt_s[0] = m
                pin(before_softmax, u, lambda z: mt_s[z, 0:8, :])
                pin(before_softmax, u, lambda z: st_s[z, 0:8, 0:LANES])
                return
            m = jnp.max(jnp.maximum(m, mt_s[z]), axis=1, keepdims=True)
            steps = n_tail // 16

            def scores(i):
                return st_s[z, 16 * i:16 * i + 16, :]

            loaded = [scores(i) for i in range(tail_ahead)]
            for i in range(steps):
                e = jnp.exp2((loaded.pop(0) - m[16 * i:16 * i + 16]) * c)
                l = e[:, 0:LANES]
                for j in range(LANES, sk, LANES):
                    l = l + e[:, j:j + LANES]
                inv_l = 1.0 / jnp.sum(l, axis=1, keepdims=True)
                pt_s[h % 2][0, 8 * i:8 * i + 8, :] = _as_u32(
                    (e * inv_l).astype(jnp.bfloat16))
                if i + tail_ahead < steps:
                    st_s[0, n_tail:n_tail + 16, 0:LANES] = jnp.broadcast_to(
                        inv_l, (16, LANES))
                    loaded.append(scores(i + tail_ahead))
            pin(before_softmax, u + 2,
                lambda z: _as_f32(pt_s[h % 2][z, 0:8, 0:LANES]))

        def tail_pv(h, part, u):
            z = zero()
            p = _as_bf16(pt_s[h % 2][z])
            d0, d1 = (0, LANES) if part == 0 else (LANES, d)
            vt = _as_bf16(v_s[h][z, d0 // 2:d1 // 2, :])
            if part == 0:
                o = lax.dot_general(p, vt, NT_DIMS, preferred_element_type=jnp.float32)
                o = o.astype(o_hbm.dtype).T
            else:
                o = lax.dot_general(vt, p, NT_DIMS, preferred_element_type=jnp.float32)
                o = o.astype(o_hbm.dtype)
            o_out[h][out_slot, d0:d1, tail0:sq] = o
            pin(before_softmax, u,
                lambda z: _as_f32(o_out[h][out_slot + z, d0:d0 + 16, 0:LANES]))

        for j in range(key_blocks):
            prepare_v(0, slot0, j)
        prepare_tail_q(0)
        weights = None
        for u in range(n * n_units):
            h, t = divmod(u, n_units)
            m = qk(u)
            if u == 0:
                tail_qk(0, 0, 1)
                tail_qk(0, 1, 1)
            else:
                pv(u - 1, *weights)
            prepare_next_head(u)
            weights = softmax(u, m)
            for part in range(2):
                if h > 0 and t == TAIL_QK_AT[part]:
                    tail_qk(h, part, u + 1)
                if t == (n_units - 1 if h == n - 1 else TAIL_PV_AT[part]):
                    tail_pv(h, part, u + 1)
        pv(n * n_units - 1, *weights)

    first_k = pltpu.make_async_copy(k_hbm.at[0], k_in.at[2 * group - 1], in_sem.at[1])
    first_k.start()
    start_inputs(0, ramp, group, in_sem.at[2])
    first_k.wait()
    for j in range(key_blocks):
        prepare_k(0, 2 * group - 1, j)

    def ramp_step(it, carry):
        half = it % 2

        @pl.when(it + 1 < group)
        def _():
            start_inputs((it + 1) * ramp, ramp, group + (1 - half) * ramp,
                         in_sem.at[3 - half])

        start_inputs(ramp_heads + it, 1, it, in_sem.at[0])
        wait_inputs(ramp, group + half * ramp, in_sem.at[2 + half])

        @pl.when(it >= 2)
        def _():
            wait_outputs(ramp, 3 + half, (it - 2) * ramp)

        run_group(it, ramp, it * ramp, group + half * ramp, 3 + half)
        return carry

    def main_step(it, carry):
        half = it % 2
        head0 = ramp_heads + it * group

        @pl.when(it + 1 < n_groups)
        def _():
            start_inputs(head0 + group, group, (1 - half) * group, in_sem.at[1 - half])

        wait_inputs(group, half * group, in_sem.at[half])

        @pl.when(it >= 2)
        def _():
            wait_outputs(group, 1 + half, head0 - 2 * group)

        run_group(it, group, head0, half * group, 1 + half)
        return carry

    lax.fori_loop(0, group, ramp_step, 0)
    lax.fori_loop(0, n_groups, main_step, 0)
    for it in (group - 2, group - 1):
        wait_outputs(ramp, 3 + it % 2, it * ramp)
    for it in (n_groups - 2, n_groups - 1):
        wait_outputs(group, 1 + it % 2, ramp_heads + it * group)


def _attention(q, k, v, interpret=False, **overrides):
    cfg = {**DEFAULTS, **overrides}
    group, ramp = cfg["group"], cfg["ramp"]
    b, hq, sq, d = q.shape
    hkv, sk = k.shape[1], k.shape[2]
    if hkv != hq:
        k = jnp.repeat(k, hq // hkv, axis=1)
        v = jnp.repeat(v, hq // hkv, axis=1)
    n_heads, n_tail = b * hq, sq % LANES
    assert (sq // LANES, sk) == (6, 4 * LANES) and LANES < d <= 2 * LANES
    assert n_tail % 16 == 0 and n_tail // 16 >= cfg["tail_ahead"]
    assert n_heads % group == 0 and n_heads >= group * (ramp + 2)
    assert ramp >= 2 and group >= 2 * ramp

    def kernel_function(*refs):
        _attention_kernel(*refs, **cfg)

    vmem, bf16, u32, f32 = pltpu.VMEM, jnp.bfloat16, jnp.uint32, jnp.float32
    out = pl.pallas_call(
        kernel_function,
        in_specs=[pl.BlockSpec(memory_space=pl.ANY)] * 3,
        out_specs=pl.BlockSpec(memory_space=pl.ANY),
        out_shape=jax.ShapeDtypeStruct((n_heads, d, sq), q.dtype),
        scratch_shapes=[
            vmem((2 * group, d, sq), bf16),
            vmem((2 * group, d, sk), bf16),
            vmem((2 * group, d, sk), bf16),
            [vmem((5 if h < ramp else 3, d, sq), bf16)
             for h in range(group)],
            [vmem((1, sk // 2, d), u32)] * group,
            vmem((1, d // 2, sk), u32),
            [vmem((1, d // 2, sk), u32)] * group,
            [vmem((1, sk + 64, LANES), f32)] * 2,
            [vmem((1, n_tail // 2, d), u32)] * 2,
            vmem((1, n_tail + 16, sk), f32),
            vmem((1, n_tail, LANES), f32),
            [vmem((1, n_tail // 2, sk), u32)] * 2,
            pltpu.SemaphoreType.DMA((4,)),
            pltpu.SemaphoreType.DMA((5,)),
        ],
        compiler_params=pltpu.CompilerParams(
            vmem_limit_bytes=100 * 1024 * 1024, disable_bounds_checks=True),
        interpret=interpret,
    )(jnp.swapaxes(q, 2, 3).reshape(n_heads, d, sq),
      jnp.swapaxes(k, 2, 3).reshape(n_heads, d, sk),
      jnp.swapaxes(v, 2, 3).reshape(n_heads, d, sk))
    return jnp.swapaxes(out.reshape(b, hq, d, sq), 2, 3)


@jax.jit
def pallas_standalone__gqa_softmax__near_ridge_kernel(
    q: jax.Array,
    k: jax.Array,
    v: jax.Array,
):
    return _attention(q, k, v)
```

```python
import math

import jax
import jax.numpy as jnp
from jax import lax
import jax.experimental.pallas as pl
import jax.experimental.pallas.tpu as pltpu

LANES = 128
NT_DIMS = (((1,), (1,)), ((), ()))

DEFAULTS = dict(
    group=16,
    ramp=2,
    chunk=32,
    ahead=4,
    tail_ahead=3,
    k_at=(0, 1, 3, 4),
    v_at=(0, 2, 3, 4),
    q_at=5,
    early=208,
    dma_lag=1,
)
TAIL_QK_AT = (0, 1)
TAIL_PV_AT = (4, 5)


def _as_u32(x):
    return pltpu.bitcast(x, jnp.uint32)


def _as_f32(x):
    return pltpu.bitcast(x, jnp.float32)


def _as_bf16(x):
    return pltpu.bitcast(x, jnp.bfloat16)


def _attention_kernel(q_hbm, k_hbm, v_hbm, o_hbm,
                      q_in, k_in, v_in, o_out, k_s, kt_s, v_s, s_s,
                      qt_s, st_s, mt_s, pt_s, q_sem, k_sem, v_sem, out_sem,
                      *, group, ramp, chunk, ahead, tail_ahead,
                      k_at, v_at, q_at, dma_lag, early):
    n_heads, d, sq = q_hbm.shape
    sk = k_hbm.shape[2]
    c = d ** -0.5 * math.log2(math.e)
    n_units = sq // LANES
    tail0 = n_units * LANES
    n_tail = sq - tail0
    key_blocks = sk // LANES
    ramp_heads = group * ramp
    n_groups = (n_heads - ramp_heads) // group

    def start_inputs(head, n, slot, batch):
        last = jnp.minimum(head + n, n_heads - 1)
        pltpu.make_async_copy(k_hbm.at[last], k_in.at[slot + n - 1],
                              k_sem.at[batch]).start()
        if n > 1:
            pltpu.make_async_copy(k_hbm.at[pl.ds(head + 1, n - 1)],
                                  k_in.at[pl.ds(slot, n - 1)], k_sem.at[batch]).start()
        for src, dst, sem in ((q_hbm, q_in, q_sem), (v_hbm, v_in, v_sem)):
            pltpu.make_async_copy(src.at[pl.ds(head, n)],
                                  dst.at[pl.ds(slot, n)], sem.at[batch]).start()

    def wait_inputs(n, slot, batch):
        for buf, sem in ((k_in, k_sem), (q_in, q_sem), (v_in, v_sem)):
            filled = buf.at[pl.ds(slot, n)]
            pltpu.make_async_copy(filled, filled, sem.at[batch]).wait()

    def output_copy(h, slot, head):
        return pltpu.make_async_copy(o_out[h].at[slot], o_hbm.at[head],
                                     out_sem.at[slot])

    def wait_outputs(n, slot, head):
        for h in range(n):
            output_copy(h, slot, head + h).wait()

    def prepare_k(h, slot, j):
        kt = k_in[slot, :, j * LANES:(j + 1) * LANES]
        k_s[h][0, j * LANES // 2:(j + 1) * LANES // 2, :] = _as_u32(kt.T)
        if h == 0:
            kt_s[0, :, j * LANES:(j + 1) * LANES] = _as_u32(kt)

    def prepare_v(h, slot, j):
        v_s[h][0, :, j * LANES:(j + 1) * LANES] = _as_u32(
            v_in[slot, :, j * LANES:(j + 1) * LANES])

    def run_group(it, n, head0, slot0, out_slot):
        n_zeros = 0

        def zero():
            nonlocal n_zeros
            n_zeros += 1
            return lax.shift_right_logical(it + n_zeros, 24)

        before_softmax, before_qk_end = {}, {}

        def pin(where, unit, load):
            where.setdefault(unit, []).append(load)

        def qk(u):
            h, t = divmod(u, n_units)
            buf, z = s_s[u % 2], zero()
            qt = q_in[slot0 + h, :, t * LANES:(t + 1) * LANES]
            half = sk // 2
            parts, m = [], None
            for j in range(2):
                k = _as_bf16(k_s[h][z, j * half // 2:(j + 1) * half // 2, :])
                s = jnp.dot(k, qt, preferred_element_type=jnp.float32)
                mj = jnp.max(s.reshape(half // 8, 8, LANES), axis=0)
                m = mj if m is None else jnp.maximum(m, mj)
                buf[0, j * half:j * half + early, :] = s[:early]
                parts.append(s[early:])
            for i, load in enumerate(before_qk_end.pop(u, [])):
                buf[z, sk + 32 + 8 * i:sk + 40 + 8 * i, :] = load(z)
            for j in range(2):
                buf[0, j * half + early:(j + 1) * half, :] = parts[j]
            return jnp.broadcast_to(jnp.max(m, axis=0, keepdims=True), (8, LANES))

        def prepare_next_head(u):
            h, t = divmod(u, n_units)
            nxt = (h + 1) % n
            for j in range(key_blocks):
                if t == k_at[j]:
                    prepare_k(nxt, slot0 + h, j)
                    pin(before_softmax, u, lambda z, j=j: _as_f32(
                        k_s[nxt][z, j * LANES // 2:j * LANES // 2 + 8, 0:LANES]))
                    if nxt == 0:
                        pin(before_softmax, u, lambda z, j=j: _as_f32(
                            kt_s[z, 0:8, j * LANES:(j + 1) * LANES]))
                if t == v_at[j] and nxt:
                    prepare_v(nxt, slot0 + nxt, j)
                    pin(before_qk_end, u + 1, lambda z, j=j: _as_f32(
                        v_s[nxt][z, 0:8, j * LANES:(j + 1) * LANES]))
            if t == q_at and nxt:
                prepare_tail_q(nxt)
                pin(before_softmax, u,
                    lambda z: _as_f32(qt_s[nxt % 2][z, 0:8, 0:LANES]))

        def softmax(u, m):
            buf, z = s_s[u % 2], zero()
            for i, load in enumerate(before_softmax.pop(u, [])):
                buf[0, sk + 8 * i:sk + 8 * i + 8, :] = load(z)
            starts = list(range(0, sk, chunk))[::-1]

            def scores(i):
                return buf[z, starts[i]:starts[i] + chunk, :]

            loaded = [scores(i) for i in range(ahead)]
            p, l = [], None
            for i in range(len(starts)):
                s = loaded.pop(0).reshape(chunk // 8, 8, LANES)
                e = jnp.exp2((s - m) * c)
                li = jnp.sum(e, axis=0)
                l = li if l is None else l + li
                p.insert(0, e.reshape(chunk, LANES))
                if i + ahead < len(starts):
                    buf[0, starts[i]:starts[i] + 8, :] = l
                    loaded.append(scores(i + ahead))
            l = jnp.sum(l, axis=0, keepdims=True)
            return jnp.concatenate(p, axis=0).astype(jnp.bfloat16), 1.0 / l

        def pv(u, p, inv_l):
            h, t = divmod(u, n_units)
            o = jnp.dot(_as_bf16(v_s[h][zero()]), p,
                        preferred_element_type=jnp.float32)
            o_out[h][out_slot, :, t * LANES:(t + 1) * LANES] = (
                o * inv_l).astype(o_hbm.dtype)
            if t == n_units - 1:
                output_copy(h, out_slot, head0 + h).start()

                def after_dma_start(z):
                    o_out[h][z, 0:16, 0:LANES] = jnp.zeros((16, LANES), o_hbm.dtype)
                    return _as_f32(o_out[h][0, 0:16, 0:LANES])

                pin(before_softmax, u + 1 + dma_lag, after_dma_start)

        def prepare_tail_q(h):
            qt_s[h % 2][0, 0:n_tail // 2] = _as_u32(q_in[slot0 + h, :, tail0:sq].T)

        def tail_qk(h, part, u):
            z, w = zero(), sk // 2
            if h == 0:
                kt = _as_bf16(kt_s[z, :, part * w:(part + 1) * w])
            else:
                kt = k_in[slot0 + h - 1, :, part * w:(part + 1) * w]
            s = jnp.dot(_as_bf16(qt_s[h % 2][z, 0:n_tail // 2]), kt,
                        preferred_element_type=jnp.float32)
            st_s[0, 0:n_tail, part * w:(part + 1) * w] = s
            m = s[:, 0:LANES]
            for j in range(LANES, w, LANES):
                m = jnp.maximum(m, s[:, j:j + LANES])
            if part == 0:
                mt_s[0, 0:n_tail] = m
                pin(before_softmax, u, lambda z: mt_s[z, 0:8, :])
                pin(before_softmax, u, lambda z: st_s[z, 0:8, 0:LANES])
                return
            m = jnp.max(jnp.maximum(m, mt_s[z, 0:n_tail]), axis=1, keepdims=True)
            steps = n_tail // 16

            def scores(i):
                return st_s[z, 16 * i:16 * i + 16, :]

            loaded = [scores(i) for i in range(tail_ahead)]
            for i in range(steps):
                e = jnp.exp2((loaded.pop(0) - m[16 * i:16 * i + 16]) * c)
                l = e[:, 0:LANES]
                for j in range(LANES, sk, LANES):
                    l = l + e[:, j:j + LANES]
                inv_l = 1.0 / jnp.sum(l, axis=1, keepdims=True)
                pt_s[h % 2][0, 8 * i:8 * i + 8, :] = _as_u32(
                    (e * inv_l).astype(jnp.bfloat16))
                if i + tail_ahead < steps:
                    st_s[0, n_tail:n_tail + 16, 0:LANES] = jnp.broadcast_to(
                        inv_l, (16, LANES))
                    loaded.append(scores(i + tail_ahead))
            pin(before_softmax, u + 2,
                lambda z: _as_f32(pt_s[h % 2][z, 0:8, 0:LANES]))

        def tail_pv(h, part, u):
            z = zero()
            p = _as_bf16(pt_s[h % 2][z])
            d0, d1 = (0, LANES) if part == 0 else (LANES, d)
            vt = _as_bf16(v_s[h][z, d0 // 2:d1 // 2, :])
            if part == 0:
                o = lax.dot_general(p, vt, NT_DIMS, preferred_element_type=jnp.float32)
                o = o.astype(o_hbm.dtype).T
            else:
                o = lax.dot_general(vt, p, NT_DIMS, preferred_element_type=jnp.float32)
                o = o.astype(o_hbm.dtype)
            o_out[h][out_slot, d0:d1, tail0:sq] = o
            pin(before_softmax, u,
                lambda z: _as_f32(o_out[h][out_slot + z, d0:d0 + 16, 0:LANES]))

        for j in range(key_blocks):
            prepare_v(0, slot0, j)
        prepare_tail_q(0)
        weights = None
        for u in range(n * n_units):
            h, t = divmod(u, n_units)
            m = qk(u)
            if u == 0:
                tail_qk(0, 0, 1)
                tail_qk(0, 1, 1)
            else:
                pv(u - 1, *weights)
            prepare_next_head(u)
            weights = softmax(u, m)
            for part in range(2):
                if h > 0 and t == TAIL_QK_AT[part]:
                    tail_qk(h, part, u + 1)
                if t == (n_units - 1 if h == n - 1 else TAIL_PV_AT[part]):
                    tail_pv(h, part, u + 1)
        pv(n * n_units - 1, *weights)

    first_k = pltpu.make_async_copy(k_hbm.at[0], k_in.at[2 * group - 1], k_sem.at[1])
    first_k.start()
    start_inputs(0, ramp, group, 2)
    first_k.wait()
    for j in range(key_blocks):
        prepare_k(0, 2 * group - 1, j)

    def ramp_step(it, carry):
        half = it % 2

        @pl.when(it + 1 < group)
        def _():
            start_inputs((it + 1) * ramp, ramp, group + (1 - half) * ramp, 3 - half)

        start_inputs(ramp_heads + it, 1, it, 0)
        wait_inputs(ramp, group + half * ramp, 2 + half)

        @pl.when(it >= 2)
        def _():
            wait_outputs(ramp, 3 + half, (it - 2) * ramp)

        run_group(it, ramp, it * ramp, group + half * ramp, 3 + half)
        return carry

    def main_step(it, carry):
        half = it % 2
        head0 = ramp_heads + it * group

        @pl.when(it + 1 < n_groups)
        def _():
            start_inputs(head0 + group, group, (1 - half) * group, 1 - half)

        wait_inputs(group, half * group, half)

        @pl.when(it >= 2)
        def _():
            wait_outputs(group, 1 + half, head0 - 2 * group)

        run_group(it, group, head0, half * group, 1 + half)
        return carry

    lax.fori_loop(0, group, ramp_step, 0)
    lax.fori_loop(0, n_groups, main_step, 0)
    for it in (group - 2, group - 1):
        wait_outputs(ramp, 3 + it % 2, it * ramp)
    for it in (n_groups - 2, n_groups - 1):
        wait_outputs(group, 1 + it % 2, ramp_heads + it * group)


def _attention(q, k, v, interpret=False, **overrides):
    cfg = {**DEFAULTS, **overrides}
    group, ramp = cfg["group"], cfg["ramp"]
    b, hq, sq, d = q.shape
    hkv, sk = k.shape[1], k.shape[2]
    if hkv != hq:
        k = jnp.repeat(k, hq // hkv, axis=1)
        v = jnp.repeat(v, hq // hkv, axis=1)
    n_heads, n_tail = b * hq, sq % LANES
    assert (sq // LANES, sk) == (6, 4 * LANES) and LANES < d <= 2 * LANES
    assert n_tail % 16 == 0 and n_tail // 16 >= cfg["tail_ahead"]
    assert n_heads % group == 0 and n_heads >= group * (ramp + 2)
    assert ramp >= 2 and group >= 2 * ramp

    def kernel_function(*refs):
        _attention_kernel(*refs, **cfg)

    vmem, bf16, u32, f32 = pltpu.VMEM, jnp.bfloat16, jnp.uint32, jnp.float32
    out = pl.pallas_call(
        kernel_function,
        in_specs=[pl.BlockSpec(memory_space=pl.ANY)] * 3,
        out_specs=pl.BlockSpec(memory_space=pl.ANY),
        out_shape=jax.ShapeDtypeStruct((n_heads, d, sq), q.dtype),
        scratch_shapes=[
            vmem((2 * group, d, sq), bf16),
            vmem((2 * group, d, sk), bf16),
            vmem((2 * group, d, sk), bf16),
            [vmem((5 if h < ramp else 3, d, sq), bf16)
             for h in range(group)],
            [vmem((1, sk // 2, d), u32)] * group,
            vmem((1, d // 2, sk), u32),
            [vmem((1, d // 2, sk), u32)] * group,
            [vmem((1, sk + 64, LANES), f32)] * 2,
            [vmem((1, n_tail // 2 + 8, d), u32)] * 2,
            vmem((1, n_tail + 16, sk), f32),
            vmem((1, n_tail + 16, LANES), f32),
            [vmem((1, n_tail // 2, sk), u32)] * 2,
            pltpu.SemaphoreType.DMA((4,)),
            pltpu.SemaphoreType.DMA((4,)),
            pltpu.SemaphoreType.DMA((4,)),
            pltpu.SemaphoreType.DMA((5,)),
        ],
        compiler_params=pltpu.CompilerParams(
            vmem_limit_bytes=100 * 1024 * 1024, disable_bounds_checks=True),
        interpret=interpret,
    )(jnp.swapaxes(q, 2, 3).reshape(n_heads, d, sq),
      jnp.swapaxes(k, 2, 3).reshape(n_heads, d, sk),
      jnp.swapaxes(v, 2, 3).reshape(n_heads, d, sk))
    return jnp.swapaxes(out.reshape(b, hq, d, sq), 2, 3)


@jax.jit
def pallas_standalone__gqa_softmax__near_ridge_kernel(
    q: jax.Array,
    k: jax.Array,
    v: jax.Array,
):
    return _attention(q, k, v)
```
